```python
import os as _os
_os.environ.setdefault("JAX_PLATFORMS", "cpu")
import jax
import jax.numpy as jnp

def _softmax(x, axis=-1):
    return jax.nn.softmax(x, axis=axis)
def _gelu(x):
    return jax.nn.gelu(x, approximate=True)
def _silu(x):
    return jax.nn.silu(x)
def _sigmoid(x):
    return jax.nn.sigmoid(x)
def _layernorm(x, axis=-1, eps=1e-5):
    m = jnp.mean(x, axis=axis, keepdims=True)
    v = jnp.var(x, axis=axis, keepdims=True)
    return (x - m) / jnp.sqrt(v + eps)
def _scatter_add(tgt, idx, src, axis=0):
    return tgt.at[idx].add(src)
def _segment_sum(src, seg, n):
    return jax.ops.segment_sum(src, seg, n)
class _Rng:
    def __init__(self, key):
        self._k = key
    def _next(self):
        self._k, sub = jax.random.split(self._k)
        return sub
    def normal(self, shape):
        return jax.random.normal(self._next(), shape, dtype=jnp.bfloat16)
    def randint(self, lo, hi, shape):
        return jax.random.randint(self._next(), shape, lo, hi, dtype=jnp.int32)
    def uniform(self, shape, lo=0.0, hi=1.0):
        return jax.random.uniform(self._next(), shape, jnp.bfloat16, lo, hi)
    def permutation(self, n):
        return jax.random.permutation(self._next(), n)


kernel_name = 'standalone__mha_block_cached__near_ridge'

def setup_inputs():
    _rng = _Rng(jax.random.key(int.from_bytes(__import__("os").urandom(4), "little")))
    _w = (lambda a: (lambda t: t.astype(jnp.bfloat16) if jnp.issubdtype(t.dtype, jnp.floating) else t)(jnp.asarray(a)))
    B, Sq, D = 16, 64, 576
    H, Sk, Dh = 32, 64, 128
    return {
        "x": _w((lambda *s: _rng.normal(s) * 0.8)(B, Sq, D)),
        "k_cache": _w((lambda *s: _rng.normal(s) * 0.8)(B, H, Sk, Dh)),
        "v_cache": _w((lambda *s: _rng.normal(s) * 0.05)(B, H, Sk, Dh)),
        "wq": _w((lambda *s: _rng.normal(s) * 0.8)(D, H * Dh) * (D ** -0.5)),
        "wo": _w((lambda *s: _rng.normal(s) * 0.05)(H * Dh, D) * ((H * Dh) ** -0.5)),
    }

def reference(x, k_cache, v_cache, wq, wo):
    B, Sq, D = x.shape
    H, Dh = 32, 128
    q = (lambda x, *d: x.transpose(*d))((x @ wq).reshape(B, Sq, H, Dh), 0, 2, 1, 3)
    scores = jnp.einsum("bhqd,bhkd->bhqk", q, k_cache) * (Dh ** -0.5)
    p = _softmax(scores, axis=-1)
    o = jnp.einsum("bhqk,bhkd->bhqd", p, v_cache)
    return (lambda x, *d: x.transpose(*d))(o, 0, 2, 1, 3).reshape(B, Sq, H * Dh) @ wo
```

```python
import functools
import jax
import jax.numpy as jnp
import jax.experimental.pallas as pl
import jax.experimental.pallas.tpu as pltpu

B, SQ, D = 16, 64, 576
H, SK, DH = 32, 64, 128
M = B * SQ


def _kernel(x_ref, k_ref, v_ref, wq_ref, wo_ref, o_ref, q_s, att_s, acc_s, *, nh):
    step = pl.program_id(0)
    c = (DH ** -0.5) * 1.4426950408889634

    q = jnp.dot(x_ref[...], wq_ref[...], preferred_element_type=jnp.float32)
    q_s[...] = (q * c).astype(jnp.bfloat16)

    row = jax.lax.broadcasted_iota(jnp.int32, (128, 128), 0)
    col = jax.lax.broadcasted_iota(jnp.int32, (128, 128), 1)
    valid = (row < 64) == (col < 64)

    for j in range(nh):
        for p in range(B // 2):
            qp = q_s[128 * p:128 * (p + 1), 128 * j:128 * (j + 1)]
            kp = k_ref[2 * p:2 * p + 2, j].reshape(128, 128)
            vp = v_ref[2 * p:2 * p + 2, j].reshape(128, 128)
            s = jax.lax.dot_general(qp, kp, (((1,), (1,)), ((), ())),
                                    preferred_element_type=jnp.float32)
            s = jnp.where(valid, s, -jnp.inf)
            m = jnp.max(s, axis=-1, keepdims=True)
            e = jnp.exp2(s - m)
            l = jnp.sum(e, axis=-1, keepdims=True)
            o = jnp.dot(e.astype(jnp.bfloat16), vp, preferred_element_type=jnp.float32)
            o = o * (1.0 / l)
            att_s[128 * p:128 * (p + 1), 128 * j:128 * (j + 1)] = o.astype(jnp.bfloat16)

    part = jnp.dot(att_s[...], wo_ref[...], preferred_element_type=jnp.float32)

    @pl.when(step == 0)
    def _():
        acc_s[...] = part

    @pl.when(step > 0)
    def _():
        acc_s[...] += part

    @pl.when(step == pl.num_programs(0) - 1)
    def _():
        o_ref[...] = acc_s[...].astype(o_ref.dtype)


@jax.jit
def pallas_standalone__mha_block_cached__near_ridge_kernel(x, k_cache, v_cache, wq, wo):
    nh = 2
    x2 = x.reshape(M, D)
    out = pl.pallas_call(
        functools.partial(_kernel, nh=nh),
        grid=(H // nh,),
        in_specs=[
            pl.BlockSpec((M, D), lambda i: (0, 0)),
            pl.BlockSpec((B, nh, SK, DH), lambda i: (0, i, 0, 0)),
            pl.BlockSpec((B, nh, SK, DH), lambda i: (0, i, 0, 0)),
            pl.BlockSpec((D, nh * DH), lambda i: (0, i)),
            pl.BlockSpec((nh * DH, D), lambda i: (i, 0)),
        ],
        out_specs=pl.BlockSpec((M, D), lambda i: (0, 0)),
        out_shape=jax.ShapeDtypeStruct((M, D), jnp.bfloat16),
        scratch_shapes=[
            pltpu.VMEM((M, nh * DH), jnp.bfloat16),
            pltpu.VMEM((M, nh * DH), jnp.bfloat16),
            pltpu.VMEM((M, D), jnp.float32),
        ],
        compiler_params=pltpu.CompilerParams(
            dimension_semantics=("arbitrary",),
            vmem_limit_bytes=64 * 1024 * 1024,
        ),
    )(x2, k_cache, v_cache, wq, wo)
    return out.reshape(B, SQ, D)
```

```python
import jax
import jax.numpy as jnp
import jax.experimental.pallas as pl
import jax.experimental.pallas.tpu as pltpu

B, SQ, D = 16, 64, 576
H, SK, DH = 32, 64, 128
M = B * SQ
NP = B // 2
DM = 512
ORDER = "BRDC"
SKEW = dict(zip("BRCD", [int(c, 16) for c in "0248"]))
AG = int("1")
N0 = 2
N0B = int("4")
N1 = (H - 4 - N0 - N0B) // 2
DSPLIT = int("2")
GL = int("4")
APS = int("1")
BF = jnp.bfloat16
F32 = jnp.float32
U32 = jnp.uint32
TN = (((0,), (0,)), ((), ()))
assert N0 + N0B + 2 * N1 + 4 == H
NMAIN = H - 4


def p2_head(i, j):
    if j < 2:
        return 14 * i + j
    if j < 4:
        return NMAIN + 2 * i + (j - 2)
    return 14 * i + (j - 2)


def _kernel(x_hbm, k_hbm, v_hbm, wq_hbm, wo_hbm, o_hbm,
            x_s, k_s, v_s, wq_s, wo_s, t_s, tt_s, wr_s, wrt_s, xr_s, acc_s, out_s,
            sem_x, sem_w0, sem_w1, sem_wt, sem_kv, sem_o, bar_sem):
    c = (DH ** -0.5) * 1.4426950408889634

    def cols(h0, n):
        return pl.ds(h0 * 128 if isinstance(h0, int) else pl.multiple_of(h0 * 128, 128), 128 * n)

    def x_copy(i):
        return pltpu.make_async_copy(x_hbm.at[pl.ds(512 * i, 512)], x_s.at[pl.ds(512 * i, 512)], sem_x.at[i])

    def w_copies(src, dst, h0, n, sem):
        return [pltpu.make_async_copy(src.at[:, cols(h0 + j, 1)], dst.at[h0 + j], sem) for j in range(n)]

    def w0_copy(i):
        return w_copies(wq_hbm, wq_s, 0, N0, sem_w0.at[0]) if i == 0 else w_copies(wq_hbm, wq_s, N0, N0B, sem_w0.at[1])

    def w1_copy(i):
        return w_copies(wq_hbm, wq_s, N0 + N0B + N1 * i, N1, sem_w1.at[i])

    def wt_copy(i):
        return w_copies(wq_hbm, wq_s, NMAIN + 2 * i, 2, sem_wt.at[i])

    def kv_copies(i):
        out = []
        for part, (h0, n) in enumerate(((14 * i, 14), (NMAIN + 2 * i, 2))):
            out.append(pltpu.make_async_copy(k_hbm.at[:, pl.ds(h0, n)], k_s.at[:, pl.ds(h0, n)], sem_kv.at[i, 3 * part]))
            out.append(pltpu.make_async_copy(v_hbm.at[:, pl.ds(h0, n)], v_s.at[:, pl.ds(h0, n)], sem_kv.at[i, 3 * part + 1]))
            out += w_copies(wo_hbm, wo_s, h0, n, sem_kv.at[i, 3 * part + 2])
        return out

    def wait_all(cps):
        for cp in cps:
            cp.wait()

    def o_copy(p):
        return pltpu.make_async_copy(out_s.at[p], o_hbm.at[pl.ds(128 * p, 128)], sem_o.at[p])

    def bar():
        pl.semaphore_signal(bar_sem, 1)
        pl.semaphore_wait(bar_sem, 1)

    groups = [[x_copy(0)], w0_copy(0), [x_copy(1)], w0_copy(1), w1_copy(0), w1_copy(1),
              wt_copy(0) + kv_copies(0), wt_copy(1) + kv_copies(1)]
    for g in groups:
        for cp in g:
            cp.start()
        bar()

    acc_s[...] = jnp.zeros_like(acc_s)

    left = jax.lax.broadcasted_iota(jnp.int32, (64, 128), 1) < 64
    left1 = jax.lax.broadcasted_iota(jnp.int32, (1, 128), 1) < 64

    def to_u32(v):
        return pltpu.bitcast(v, U32)

    def to_bf(v):
        return pltpu.bitcast(v, BF)

    def make_xr(p):
        xr = x_s[128 * p:128 * (p + 1), DM:D].astype(F32)
        z = jnp.zeros((64, 64), F32)
        top = jnp.concatenate([z, xr[:64]], axis=1)
        bot = jnp.concatenate([xr[64:], z], axis=1)
        xr_s[p] = to_u32(jnp.concatenate([top, bot], axis=0).T.astype(BF))

    def make_wr(h, dst=None):
        wr = wq_s[h, DM:D, :]
        val = to_u32(jnp.concatenate([wr, wr], axis=0).T)
        if dst is None:
            wr_s[h] = val
        else:
            wrt_s[dst] = val

    def stA(h0, nh, r0, nr, dst=None):
        for j in range(nh):
            h = h0 + j
            q = jnp.dot(x_s[r0:r0 + nr, 0:DM], wq_s[h, 0:DM, :], preferred_element_type=F32).astype(BF)
            wr2 = wr_s[h] if dst is None else wrt_s[dst]
            for i in range(nr // 128):
                p = r0 // 128 + i
                qt = to_u32(q[128 * i:128 * (i + 1), :].T)
                ref, idx = (t_s, h) if dst is None else (tt_s, dst)
                ref[idx, p, 0] = jnp.where(left, qt, wr2)
                ref[idx, p, 1] = jnp.where(left, wr2, qt)

    def a_heads(h0, n):
        j = 0
        while j < n:
            nh = min(AG, n - j)
            for jj in range(nh):
                make_wr(h0 + j + jj)
            stA(h0 + j, nh, 0, M)
            j += nh

    def stB(h, p, tidx):
        ref, idx = (t_s, h) if tidx is None else (tt_s, tidx)
        r1 = jnp.dot(k_s[2 * p, h], to_bf(ref[idx, p, 0]), preferred_element_type=F32)
        r2 = jnp.dot(k_s[2 * p + 1, h], to_bf(ref[idx, p, 1]), preferred_element_type=F32)
        s_main = jnp.where(left, r1, r2)
        g = jnp.where(left, r2, r1).astype(BF)
        return s_main, g

    def stR(h, p, sg):
        s_main, g = sg
        s = s_main + jnp.dot(g, to_bf(xr_s[p]), preferred_element_type=F32)
        m = jnp.max(s, axis=0, keepdims=True)
        e = jnp.exp2((s - m) * c)
        l = jnp.sum(e, axis=0, keepdims=True)
        r = 1.0 / l
        rt = jnp.where(left1, r, 0.0)
        rb = jnp.where(left1, 0.0, r)
        return jnp.concatenate([(e * rt).astype(BF), (e * rb).astype(BF)], axis=0)

    def stC(h, p, w):
        vp = v_s[2 * p:2 * p + 2, h].reshape(128, 128)
        ot = jax.lax.dot_general(vp, w, TN, preferred_element_type=F32)
        return ot.astype(BF)

    def stD(h, p, ot, last, last_iter):
        rows = D // DSPLIT
        parts = []
        for r in range(DSPLIT):
            sl = slice(rows * r, rows * (r + 1))
            part = acc_s[p, sl] + jnp.dot(wo_s[h, sl, :], ot, preferred_element_type=F32)
            acc_s[p, sl] = part
            parts.append(part)
        if last:
            full = parts[0] if DSPLIT == 1 else jnp.concatenate(parts, axis=0)
            out_s[p] = full.astype(BF).T

            @pl.when(last_iter)
            def _():
                o_copy(p).start()

    import contextlib
    SC = None
    scope = (lambda n: jax.named_scope(n)) if SC else (lambda n: contextlib.nullcontext())
    with scope("w_x0"):
        x_copy(0).wait(); wait_all(w0_copy(0))
    with scope("a0"):
        for h in range(N0):
            make_wr(h)
        stA(0, N0, 0, 512)
    with scope("w_x1"):
        x_copy(1).wait()
    with scope("a1"):
        for p in range(NP):
            make_xr(p)
        stA(0, N0, 512, 512)
    with scope("w_w0b"):
        wait_all(w0_copy(1))
    with scope("a0b"):
        a_heads(N0, N0B)

    def p1_body(i, carry):
        with scope("w_p1"):
            wait_all(w1_copy(i))
        with scope("p1"):
            a_heads(N0 + N0B + N1 * i, N1)
        return carry

    jax.lax.fori_loop(0, 2, p1_body, 0)

    def p2_body(i, carry):
        with scope("w_kv"):
            wait_all(wt_copy(i) + kv_copies(i))
        with scope("p2"):
            p2_main(i)
        return carry

    def p2_main(i):

        th = NMAIN + 2 * i
        make_wr(th, 0); make_wr(th + 1, 1)
        tail_pieces = [(th + j, 1, 128 * r, 128, j) for j in range(2) for r in range(NP)]
        units = [(j, p) for j in range(16 - GL) for p in range(NP)]
        units += [(j, p) for p in range(NP) for j in range(16 - GL, 16)]
        n = len(units)
        prev = dict(B=None, R="B", C="R", D="C")
        vals = {}
        for t in range(n + max(SKEW.values())):
            for _ in range(APS):
                if tail_pieces:
                    stA(*tail_pieces.pop(0))
            for s in ORDER:
                u = t - SKEW[s]
                if 0 <= u < n:
                    j, p = units[u]
                    h = p2_head(i, j)
                    inp = vals.pop((prev[s], u)) if prev[s] else None
                    if s == "B":
                        vals[(s, u)] = stB(h, p, j - 2 if 2 <= j < 4 else None)
                    elif s == "R":
                        vals[(s, u)] = stR(h, p, inp)
                    elif s == "C":
                        vals[(s, u)] = stC(h, p, inp)
                    else:
                        stD(h, p, inp, j == 15, i == 1)

    jax.lax.fori_loop(0, 2, p2_body, 0)
    with scope("w_out"):
        for p in range(NP):
            o_copy(p).wait()


@jax.jit
def pallas_standalone__mha_block_cached__near_ridge_kernel(x, k_cache, v_cache, wq, wo):
    x2 = x.reshape(M, D)
    out = pl.pallas_call(
        _kernel,
        in_specs=[pl.BlockSpec(memory_space=pl.ANY)] * 5,
        out_specs=pl.BlockSpec(memory_space=pl.ANY),
        out_shape=jax.ShapeDtypeStruct((M, D), BF),
        scratch_shapes=[
            pltpu.VMEM((M, D), BF),
            pltpu.VMEM((B, H, SK, DH), BF),
            pltpu.VMEM((B, H, SK, DH), BF),
            pltpu.VMEM((H, D, DH), BF),
            pltpu.VMEM((H, D, DH), BF),
            pltpu.VMEM((H, NP, 2, 64, 128), U32),
            pltpu.VMEM((2, NP, 2, 64, 128), U32),
            pltpu.VMEM((H, 64, 128), U32),
            pltpu.VMEM((2, 64, 128), U32),
            pltpu.VMEM((NP, 64, 128), U32),
            pltpu.VMEM((NP, D, 128), F32),
            pltpu.VMEM((NP, 128, D), BF),
            pltpu.SemaphoreType.DMA((2,)),
            pltpu.SemaphoreType.DMA((2,)),
            pltpu.SemaphoreType.DMA((2,)),
            pltpu.SemaphoreType.DMA((2,)),
            pltpu.SemaphoreType.DMA((2, 6)),
            pltpu.SemaphoreType.DMA((NP,)),
            pltpu.SemaphoreType.REGULAR,
        ],
        compiler_params=pltpu.CompilerParams(
            vmem_limit_bytes=100 * 1024 * 1024,
        ),
    )(x2, k_cache, v_cache, wq, wo.T)
    return out.reshape(B, SQ, D)
```

```python
import contextlib
import jax
import jax.numpy as jnp
import jax.experimental.pallas as pl
import jax.experimental.pallas.tpu as pltpu

B, SQ, D = 16, 64, 576
H, SK, DH = 32, 64, 128
M = B * SQ
NP = B // 2
DM = 512
ORDER = "BRDC"
SKEW = dict(zip("BRCD", [int(c, 16) for c in "0248"]))
DSPLIT = int("2")
GL = int("6")
NT = 1
NM = H // 2 - NT
NMAIN = 2 * NM
WQG = [int(t) for t in "0,2,4,10,30".split(",")]
XCH = [int(t) for t in "0,256,512,1024".split(",")]
PLAN = [dict(wait=[("x", 0), ("w", 0)], do=[(0, 0, 1)]),
        dict(wait=[("x", 1)], do=[(0, 1, 2)]),
        dict(wait=[("w", 1)], do=[(1, 0, 2)]),
        dict(wait=[("x", 2)], do=[(0, 2, 3), (1, 2, 3)], xr=True),
        dict(wait=[("w", 2)], do=[(2, 0, 3)]),
        dict(wait=[("w", 3)], do=[(3, 0, 3)])]
FENCE = [int(t) for t in "132".split(",") if t]
LASTBR = int("1")
DEFD = int("1")
DEF = int("1")
BF = jnp.bfloat16
F32 = jnp.float32
U32 = jnp.uint32
TN = (((0,), (0,)), ((), ()))
SC = None
scope = (lambda n: jax.named_scope(n)) if SC else (lambda n: contextlib.nullcontext())


def p2_head(i, j):
    if j == 0:
        return NM * i
    if j <= NT:
        return NMAIN + NT * i + (j - 1)
    return NM * i + (j - NT)


def _kernel(x_hbm, k_hbm, v_hbm, wq_hbm, wo_hbm, o_hbm,
            x_s, k_s, v_s, wq_s, wo_s, t_s, tt_s, wr_s, wrt_s, xr_s, acc_s, out_s,
            sem_p1, sem_kv, sem_o, bar_sem):
    c = (DH ** -0.5) * 1.4426950408889634
    wqg = list(zip(WQG[:-1], WQG[1:]))

    def cols(h0, n):
        return pl.ds(h0 * 128 if isinstance(h0, int) else pl.multiple_of(h0 * 128, 128), 128 * n)

    def x_copy(i, sem):
        r0, r1 = XCH[i], XCH[i + 1]
        return pltpu.make_async_copy(x_hbm.at[pl.ds(r0, r1 - r0)], x_s.at[pl.ds(r0, r1 - r0)], sem)

    def w_copies(src, dst, h0, n, sem):
        return [pltpu.make_async_copy(src.at[:, cols(h0 + j, 1)], dst.at[h0 + j], sem) for j in range(n)]

    def wait_heads(buf, h0, n, sem):
        dst = buf.at[pl.ds(h0, n)]
        pltpu.make_async_copy(dst, dst, sem).wait()

    def kv_parts(i):
        return ((NM * i, NM), (NMAIN + NT * i, NT))

    def kv_copies(i):
        out = []
        for h0, n in kv_parts(i):
            out.append(pltpu.make_async_copy(k_hbm.at[:, pl.ds(h0, n)], k_s.at[:, pl.ds(h0, n)], sem_kv.at[i]))
            out.append(pltpu.make_async_copy(v_hbm.at[:, pl.ds(h0, n)], v_s.at[:, pl.ds(h0, n)], sem_kv.at[i]))
        return out

    def start_kv(i):
        cps = w_copies(wq_hbm, wq_s, NMAIN + NT * i, NT, sem_kv.at[i]) + kv_copies(i)
        for h0, n in kv_parts(i):
            cps += w_copies(wo_hbm, wo_s, h0, n, sem_kv.at[i])
        for cp in cps:
            cp.start()

    def wait_kv(i):
        wait_heads(wq_s, NMAIN + NT * i, NT, sem_kv.at[i])
        for h0, n in kv_parts(i):
            wait_heads(wo_s, h0, n, sem_kv.at[i])
        for cp in kv_copies(i):
            cp.wait()

    def o_copy(p):
        return pltpu.make_async_copy(out_s.at[p], o_hbm.at[pl.ds(128 * p, 128)], sem_o)

    def bar():
        pl.semaphore_signal(bar_sem, 1)
        pl.semaphore_wait(bar_sem, 1)

    for k, step in enumerate(PLAN):
        for kind, idx in step["wait"]:
            if kind == "x":
                x_copy(idx, sem_p1.at[k]).start()
            else:
                a, b = wqg[idx]
                for cp in w_copies(wq_hbm, wq_s, a, b - a, sem_p1.at[k]):
                    cp.start()
            bar()
    start_kv(0)
    bar()
    start_kv(1)

    acc_s[...] = jnp.zeros_like(acc_s)

    left = jax.lax.broadcasted_iota(jnp.int32, (64, 128), 1) < 64
    left1 = jax.lax.broadcasted_iota(jnp.int32, (1, 128), 1) < 64

    def to_u32(v):
        return pltpu.bitcast(v, U32)

    def to_bf(v):
        return pltpu.bitcast(v, BF)

    def make_xr(p):
        xr = x_s[128 * p:128 * (p + 1), DM:D].astype(F32)
        z = jnp.zeros((64, 64), F32)
        top = jnp.concatenate([z, xr[:64]], axis=1)
        bot = jnp.concatenate([xr[64:], z], axis=1)
        xr_s[p] = to_u32(jnp.concatenate([top, bot], axis=0).T.astype(BF))

    def make_wr(h, dst=None):
        wr = wq_s[h, DM:D, :]
        val = to_u32(jnp.concatenate([wr, wr], axis=0).T)
        if dst is None:
            wr_s[h] = val
        else:
            wrt_s[dst] = val

    def epiA(h, r0, q, dst=None):
        wr2 = wr_s[h] if dst is None else wrt_s[dst]
        for i in range(q.shape[0] // 128):
            p = r0 // 128 + i
            qt = to_u32(q[128 * i:128 * (i + 1), :].T)
            ref, idx = (t_s, h) if dst is None else (tt_s, dst)
            ref[idx, p, 0] = jnp.where(left, qt, wr2)
            ref[idx, p, 1] = jnp.where(left, wr2, qt)

    def mmA(h, r0, nr):
        return jnp.dot(x_s[r0:r0 + nr, 0:DM], wq_s[h, 0:DM, :], preferred_element_type=F32).astype(BF)

    def stA(h, r0, nr, dst=None):
        epiA(h, r0, mmA(h, r0, nr), dst)

    pending = []

    def flush():
        while pending:
            epiA(*pending.pop(0))

    def stA_defer(h, r0, nr):
        nd = 128 * DEF
        if nr > nd:
            stA(h, r0, nr - nd)
        pending.append((h, r0 + nr - nd, mmA(h, r0 + nr - nd, nd)))

    def stB(h, p, tidx):
        ref, idx = (t_s, h) if tidx is None else (tt_s, tidx)
        r1 = jnp.dot(k_s[2 * p, h], to_bf(ref[idx, p, 0]), preferred_element_type=F32)
        r2 = jnp.dot(k_s[2 * p + 1, h], to_bf(ref[idx, p, 1]), preferred_element_type=F32)
        s_main = jnp.where(left, r1, r2)
        g = jnp.where(left, r2, r1).astype(BF)
        return s_main, g

    def stR(h, p, sg):
        s_main, g = sg
        s = s_main + jnp.dot(g, to_bf(xr_s[p]), preferred_element_type=F32)
        m = jnp.max(s, axis=0, keepdims=True)
        e = jnp.exp2((s - m) * c)
        l = jnp.sum(e, axis=0, keepdims=True)
        r = 1.0 / l
        rt = jnp.where(left1, r, 0.0)
        rb = jnp.where(left1, 0.0, r)
        return jnp.concatenate([(e * rt).astype(BF), (e * rb).astype(BF)], axis=0)

    def stC(h, p, w):
        vp = v_s[2 * p:2 * p + 2, h].reshape(128, 128)
        ot = jax.lax.dot_general(vp, w, TN, preferred_element_type=F32)
        return ot.astype(BF)

    def stD_mm(h, ot):
        rows = D // DSPLIT
        return [jnp.dot(wo_s[h, rows * r:rows * (r + 1), :], ot, preferred_element_type=F32) for r in range(DSPLIT)]

    def stD_acc(p, prods, last, last_iter):
        rows = D // DSPLIT
        parts = []
        for r in range(DSPLIT):
            sl = slice(rows * r, rows * (r + 1))
            part = acc_s[p, sl] + prods[r]
            acc_s[p, sl] = part
            parts.append(part)
        if last:
            if p >= NP - LASTBR:
                @pl.when(last_iter)
                def _():
                    out_s[p] = acc_s[p].astype(BF).T
                    o_copy(p).start()
            else:
                out_s[p] = jnp.concatenate(parts, axis=0).astype(BF).T

                @pl.when(last_iter)
                def _():
                    o_copy(p).start()

    for k, step in enumerate(PLAN):
        with scope(f"w_s{k}"):
            for kind, idx in step["wait"]:
                if kind == "x":
                    x_copy(idx, sem_p1.at[k]).wait()
                else:
                    a, b = wqg[idx]
                    wait_heads(wq_s, a, b - a, sem_p1.at[k])
        with scope(f"s{k}"):
            flush()
            if step.get("xr"):
                for p in range(NP):
                    make_xr(p)
            items = []
            for (g, c0, c1) in step["do"]:
                for h in range(*wqg[g]):
                    items.append((h, XCH[c0], XCH[c1] - XCH[c0]))
            made = set()
            for n, (h, r0, nr) in enumerate(items):
                if ("w", [g for g in range(len(wqg)) if wqg[g][0] <= h < wqg[g][1]][0]) in step["wait"] and h not in made:
                    made.add(h)
                    make_wr(h)
                defer = DEF and n == len(items) - 1 and k < len(PLAN) - 1
                (stA_defer if defer else stA)(h, r0, nr)

    def p2_main(i):
        th = NMAIN + NT * i
        for j in range(NT):
            make_wr(th + j, j)
        tail_pieces = [(th + j, 128 * r, 128, j) for j in range(NT) for r in range(NP)]
        units = [(j, p) for j in range(16 - GL) for p in range(NP)]
        units += [(j, p) for p in range(NP) for j in range(16 - GL, 16)]
        n = len(units)
        prev = dict(B=None, R="B", C="R", D="C")
        vals = {}
        pend_acc = []
        for t in range(n + max(SKEW.values())):
            if t in FENCE:
                bar()
                while pend_acc:
                    stD_acc(*pend_acc.pop(0))
            if tail_pieces:
                stA(*tail_pieces.pop(0))
            for s in ORDER:
                u = t - SKEW[s]
                if 0 <= u < n:
                    j, p = units[u]
                    h = p2_head(i, j)
                    inp = vals.pop((prev[s], u)) if prev[s] else None
                    if s == "B":
                        vals[(s, u)] = stB(h, p, j - 1 if 1 <= j <= NT else None)
                    elif s == "R":
                        vals[(s, u)] = stR(h, p, inp)
                    elif s == "C":
                        vals[(s, u)] = stC(h, p, inp)
                    else:
                        args = (p, stD_mm(h, inp), j == 15, i == 1)
                        if any(f - DEFD <= t < f for f in FENCE):
                            pend_acc.append(args)
                        else:
                            stD_acc(*args)

    def p2_body(i, carry):
        with scope("w_kv"):
            wait_kv(i)
        with scope("p2"):
            p2_main(i)
        return carry

    jax.lax.fori_loop(0, 2, p2_body, 0)
    with scope("w_out"):
        for p in range(NP):
            o_copy(p).wait()


@jax.jit
def pallas_standalone__mha_block_cached__near_ridge_kernel(x, k_cache, v_cache, wq, wo):
    x2 = x.reshape(M, D)
    out = pl.pallas_call(
        _kernel,
        in_specs=[pl.BlockSpec(memory_space=pl.ANY)] * 5,
        out_specs=pl.BlockSpec(memory_space=pl.ANY),
        out_shape=jax.ShapeDtypeStruct((M, D), BF),
        scratch_shapes=[
            pltpu.VMEM((M, D), BF),
            pltpu.VMEM((B, H, SK, DH), BF),
            pltpu.VMEM((B, H, SK, DH), BF),
            pltpu.VMEM((H, D, DH), BF),
            pltpu.VMEM((H, D, DH), BF),
            pltpu.VMEM((H, NP, 2, 64, 128), U32),
            pltpu.VMEM((NT, NP, 2, 64, 128), U32),
            pltpu.VMEM((H, 64, 128), U32),
            pltpu.VMEM((NT, 64, 128), U32),
            pltpu.VMEM((NP, 64, 128), U32),
            pltpu.VMEM((NP, D, 128), F32),
            pltpu.VMEM((NP, 128, D), BF),
            pltpu.SemaphoreType.DMA((len(PLAN),)),
            pltpu.SemaphoreType.DMA((2,)),
            pltpu.SemaphoreType.DMA,
            pltpu.SemaphoreType.REGULAR,
        ],
        compiler_params=pltpu.CompilerParams(
            vmem_limit_bytes=100 * 1024 * 1024,
        ),
    )(x2, k_cache, v_cache, wq, wo.T)
    return out.reshape(B, SQ, D)
```

```python
import jax
import jax.numpy as jnp
import jax.experimental.pallas as pl
import jax.experimental.pallas.tpu as pltpu

B, SQ, D = 16, 64, 576
H, SK, DH = 32, 64, 128
M = B * SQ
NP = B // 2
DM = 512
NM = H // 2 - 1
NMAIN = 2 * NM

WQG = (0, 2, 4, 10, 30)
XCH = (0, 256, 512, 1024)
PLAN = (
    dict(wait=(("x", 0), ("w", 0)), do=((0, 0, 1),)),
    dict(wait=(("x", 1),), do=((0, 1, 2),)),
    dict(wait=(("w", 1),), do=((1, 0, 2),)),
    dict(wait=(("x", 2),), do=((0, 2, 3), (1, 2, 3)), xr=True),
    dict(wait=(("w", 2),), do=((2, 0, 3),)),
    dict(wait=(("w", 3),), do=((3, 0, 3),)),
)
DEFER = 256
ORDER = "BRDC"
SKEW = dict(B=0, R=2, C=4, D=8)
DSPLIT = 2
GL = 8
FENCE = 132

BF = jnp.bfloat16
F32 = jnp.float32
U32 = jnp.uint32
TN = (((0,), (0,)), ((), ()))


def _p2_head(i, j):
    if j == 0:
        return NM * i
    if j == 1:
        return NMAIN + i
    return NM * i + (j - 1)


def _kernel(x_hbm, k_hbm, v_hbm, wq_hbm, wo_hbm, o_hbm,
            x_s, k_s, v_s, wq_s, wqt_s, wo_s, t_s, tt_s, wr_s, wrt_s, xr_s, acc_s, out_s,
            sem_p1, sem_kv, sem_o, bar_sem):
    c = (DH ** -0.5) * 1.4426950408889634
    wqg = list(zip(WQG[:-1], WQG[1:]))

    def x_copy(i, sem):
        r0, r1 = XCH[i], XCH[i + 1]
        return pltpu.make_async_copy(x_hbm.at[pl.ds(r0, r1 - r0)], x_s.at[pl.ds(r0, r1 - r0)], sem)

    def w_copies(src, dst, h0, n, sem):
        return [pltpu.make_async_copy(src.at[:, pl.ds(128 * (h0 + j), 128)], dst.at[h0 + j], sem)
                for j in range(n)]

    def wait_heads(buf, h0, n, sem):
        dst = buf.at[pl.ds(h0, n)]
        pltpu.make_async_copy(dst, dst, sem).wait()

    def wq_copy(g, sem):
        a, b = wqg[g]
        cs = pl.ds(128 * a, 128 * (b - a))
        return pltpu.make_async_copy(wq_hbm.at[:, cs], wq_s.at[:, cs], sem)

    def kv_parts(i):
        return ((NM * i, NM), (NMAIN + i, 1))

    def kv_copies(i):
        out = []
        for h0, n in kv_parts(i):
            out.append(pltpu.make_async_copy(k_hbm.at[:, pl.ds(h0, n)], k_s.at[:, pl.ds(h0, n)], sem_kv.at[i]))
            out.append(pltpu.make_async_copy(v_hbm.at[:, pl.ds(h0, n)], v_s.at[:, pl.ds(h0, n)], sem_kv.at[i]))
        return out

    def wqt_copy(i):
        c0 = 128 * (NMAIN + i)
        if not isinstance(i, int):
            c0 = pl.multiple_of(c0, 128)
        return pltpu.make_async_copy(wq_hbm.at[:, pl.ds(c0, 128)], wqt_s.at[i], sem_kv.at[i])

    def start_kv(i):
        cps = [wqt_copy(i)] + kv_copies(i)
        for h0, n in kv_parts(i):
            cps += w_copies(wo_hbm, wo_s, h0, n, sem_kv.at[i])
        for cp in cps:
            cp.start()

    def wait_kv(i):
        wqt_copy(i).wait()
        for h0, n in kv_parts(i):
            wait_heads(wo_s, h0, n, sem_kv.at[i])
        for cp in kv_copies(i):
            cp.wait()

    def o_copy(p):
        return pltpu.make_async_copy(out_s.at[p], o_hbm.at[pl.ds(128 * p, 128)], sem_o)

    def fence():
        pl.semaphore_signal(bar_sem, 1)
        pl.semaphore_wait(bar_sem, 1)

    for k, step in enumerate(PLAN):
        for kind, idx in step["wait"]:
            if kind == "x":
                x_copy(idx, sem_p1.at[k]).start()
            else:
                wq_copy(idx, sem_p1.at[k]).start()
            fence()
    start_kv(0)
    fence()
    start_kv(1)

    acc_s[...] = jnp.zeros_like(acc_s)

    left = jax.lax.broadcasted_iota(jnp.int32, (64, 128), 1) < 64
    left1 = jax.lax.broadcasted_iota(jnp.int32, (1, 128), 1) < 64

    def to_u32(v):
        return pltpu.bitcast(v, U32)

    def to_bf(v):
        return pltpu.bitcast(v, BF)

    def make_xr(p):
        xr = x_s[128 * p:128 * (p + 1), DM:D].astype(F32)
        z = jnp.zeros((64, 64), F32)
        top = jnp.concatenate([z, xr[:64]], axis=1)
        bot = jnp.concatenate([xr[64:], z], axis=1)
        xr_s[p] = to_u32(jnp.concatenate([top, bot], axis=0).T.astype(BF))

    def wq_rows(h, r0, r1, tail):
        return wqt_s[h, r0:r1, :] if tail else wq_s[r0:r1, 128 * h:128 * (h + 1)]

    def make_wr(h, tail=False):
        wr = wq_rows(h, DM, D, tail)
        val = to_u32(jnp.concatenate([wr, wr], axis=0).T)
        if tail:
            wrt_s[...] = val
        else:
            wr_s[h] = val

    def mm_a(h, r0, nr, tail=False):
        return jnp.dot(x_s[r0:r0 + nr, 0:DM], wq_rows(h, 0, DM, tail), preferred_element_type=F32).astype(BF)

    def epi_a(h, r0, q, tail=False):
        wr2 = wrt_s[...] if tail else wr_s[h]
        for i in range(q.shape[0] // 128):
            p = r0 // 128 + i
            qt = to_u32(q[128 * i:128 * (i + 1), :].T)
            t1 = jnp.where(left, qt, wr2)
            t2 = jnp.where(left, wr2, qt)
            if tail:
                tt_s[p, 0] = t1
                tt_s[p, 1] = t2
            else:
                t_s[h, p, 0] = t1
                t_s[h, p, 1] = t2

    def st_a(h, r0, nr, tail=False):
        epi_a(h, r0, mm_a(h, r0, nr, tail), tail)

    def st_b(h, p, tail):
        t1, t2 = (tt_s[p, 0], tt_s[p, 1]) if tail else (t_s[h, p, 0], t_s[h, p, 1])
        r1 = jnp.dot(k_s[2 * p, h], to_bf(t1), preferred_element_type=F32)
        r2 = jnp.dot(k_s[2 * p + 1, h], to_bf(t2), preferred_element_type=F32)
        return jnp.where(left, r1, r2), jnp.where(left, r2, r1).astype(BF)

    def st_r(p, sg):
        s_main, g = sg
        s = s_main + jnp.dot(g, to_bf(xr_s[p]), preferred_element_type=F32)
        m = jnp.max(s, axis=0, keepdims=True)
        e = jnp.exp2((s - m) * c)
        r = 1.0 / jnp.sum(e, axis=0, keepdims=True)
        rt = jnp.where(left1, r, 0.0)
        rb = jnp.where(left1, 0.0, r)
        return jnp.concatenate([(e * rt).astype(BF), (e * rb).astype(BF)], axis=0)

    def st_c(h, p, w):
        vp = v_s[2 * p:2 * p + 2, h].reshape(128, 128)
        return jax.lax.dot_general(vp, w, TN, preferred_element_type=F32).astype(BF)

    def st_d_mm(h, ot):
        rows = D // DSPLIT
        return [jnp.dot(wo_s[h, rows * r:rows * (r + 1), :], ot, preferred_element_type=F32)
                for r in range(DSPLIT)]

    def st_d_acc(p, prods, last, last_iter):
        rows = D // DSPLIT
        parts = []
        for r in range(DSPLIT):
            sl = slice(rows * r, rows * (r + 1))
            part = acc_s[p, sl] + prods[r]
            acc_s[p, sl] = part
            parts.append(part)
        if not last:
            return
        if p == NP - 1:
            @pl.when(last_iter)
            def _():
                out_s[p] = acc_s[p].astype(BF).T
                o_copy(p).start()
        else:
            out_s[p] = jnp.concatenate(parts, axis=0).astype(BF).T

            @pl.when(last_iter)
            def _():
                o_copy(p).start()

    pending = []
    for k, step in enumerate(PLAN):
        for kind, idx in step["wait"]:
            if kind == "x":
                x_copy(idx, sem_p1.at[k]).wait()
            else:
                wq_copy(idx, sem_p1.at[k]).wait()
        while pending:
            epi_a(*pending.pop(0))
        if step.get("xr"):
            for p in range(NP):
                make_xr(p)
        items = [(g, h, XCH[c0], XCH[c1] - XCH[c0])
                 for (g, c0, c1) in step["do"] for h in range(*wqg[g])]
        for n, (g, h, r0, nr) in enumerate(items):
            if ("w", g) in step["wait"]:
                make_wr(h)
            if n == len(items) - 1 and k < len(PLAN) - 1:
                if nr > DEFER:
                    st_a(h, r0, nr - DEFER)
                r1 = r0 + nr - DEFER
                pending.append((h, r1, mm_a(h, r1, DEFER)))
            else:
                st_a(h, r0, nr)

    def p2_body(i, carry):
        wait_kv(i)
        last_iter = i == 1
        make_wr(i, tail=True)
        units = [(j, p) for j in range(16 - GL) for p in range(NP)]
        units += [(j, p) for p in range(NP) for j in range(16 - GL, 16)]
        n = len(units)
        vals = {}
        deferred = []
        for t in range(n + SKEW["D"]):
            if t == FENCE:
                fence()
                while deferred:
                    st_d_acc(*deferred.pop(0))
            if t < NP:
                st_a(i, 128 * t, 128, tail=True)
            for s in ORDER:
                u = t - SKEW[s]
                if not 0 <= u < n:
                    continue
                j, p = units[u]
                h = _p2_head(i, j)
                if s == "B":
                    vals["B", u] = st_b(h, p, j == 1)
                elif s == "R":
                    vals["R", u] = st_r(p, vals.pop(("B", u)))
                elif s == "C":
                    vals["C", u] = st_c(h, p, vals.pop(("R", u)))
                else:
                    args = (p, st_d_mm(h, vals.pop(("C", u))), j == 15, last_iter)
                    if t == FENCE - 1:
                        deferred.append(args)
                    else:
                        st_d_acc(*args)
        return carry

    jax.lax.fori_loop(0, 2, p2_body, 0)
    for p in range(NP):
        o_copy(p).wait()


@jax.jit
def pallas_standalone__mha_block_cached__near_ridge_kernel(x, k_cache, v_cache, wq, wo):
    out = pl.pallas_call(
        _kernel,
        in_specs=[pl.BlockSpec(memory_space=pl.ANY)] * 5,
        out_specs=pl.BlockSpec(memory_space=pl.ANY),
        out_shape=jax.ShapeDtypeStruct((M, D), BF),
        scratch_shapes=[
            pltpu.VMEM((M, D), BF),
            pltpu.VMEM((B, H, SK, DH), BF),
            pltpu.VMEM((B, H, SK, DH), BF),
            pltpu.VMEM((D, NMAIN * DH), BF),
            pltpu.VMEM((2, D, DH), BF),
            pltpu.VMEM((H, D, DH), BF),
            pltpu.VMEM((H, NP, 2, 64, 128), U32),
            pltpu.VMEM((NP, 2, 64, 128), U32),
            pltpu.VMEM((H, 64, 128), U32),
            pltpu.VMEM((64, 128), U32),
            pltpu.VMEM((NP, 64, 128), U32),
            pltpu.VMEM((NP, D, 128), F32),
            pltpu.VMEM((NP, 128, D), BF),
            pltpu.SemaphoreType.DMA((len(PLAN),)),
            pltpu.SemaphoreType.DMA((2,)),
            pltpu.SemaphoreType.DMA,
            pltpu.SemaphoreType.REGULAR,
        ],
        compiler_params=pltpu.CompilerParams(vmem_limit_bytes=100 * 1024 * 1024),
    )(x.reshape(M, D), k_cache, v_cache, wq, wo.T)
    return out.reshape(B, SQ, D)
```

```python
import jax
import jax.numpy as jnp
import jax.experimental.pallas as pl
import jax.experimental.pallas.tpu as pltpu

B, SQ, D = 16, 64, 576
H, SK, DH = 32, 64, 128
M = B * SQ
NP = B // 2
DM = 512
NM = H // 2 - 1
NMAIN = 2 * NM

WQG = (0, 2, 4, 10, 30)
XCH = (0, 256, 512, 1024)
PLAN = (
    dict(wait=(("x", 0), ("w", 0)), do=((0, 0, 1),)),
    dict(wait=(("x", 1),), do=((0, 1, 2),)),
    dict(wait=(("w", 1),), do=((1, 0, 2),)),
    dict(wait=(("x", 2),), do=((0, 2, 3), (1, 2, 3)), xr=True),
    dict(wait=(("w", 2),), do=((2, 0, 3),)),
    dict(wait=(("w", 3),), do=((3, 0, 3),)),
)
DEFER = 256
LATE = 256
ORDER = "RBDC"
SKEW = dict(B=0, R=2, C=4, D=8)
DSPLIT = 2
GL = 8
FENCE = 132

BF = jnp.bfloat16
F32 = jnp.float32
U32 = jnp.uint32
TN = (((0,), (0,)), ((), ()))


def _p2_head(i, j):
    if j == 0:
        return NM * i
    if j == 1:
        return NMAIN + i
    return NM * i + (j - 1)


def _kernel(x_hbm, k_hbm, v_hbm, wq_hbm, wo_hbm, o_hbm,
            x_s, k_s, v_s, wq_s, wqt_s, wo_s, t_s, tt_s, q2_s, tt2_s, wr_s, wrt_s, xr_s, acc_s, out_s,
            sem_p1, sem_kv, sem_o, bar_sem):
    c = (DH ** -0.5) * 1.4426950408889634
    wqg = list(zip(WQG[:-1], WQG[1:]))

    def x_copy(i, sem):
        r0, r1 = XCH[i], XCH[i + 1]
        return pltpu.make_async_copy(x_hbm.at[pl.ds(r0, r1 - r0)], x_s.at[pl.ds(r0, r1 - r0)], sem)

    def w_copies(src, dst, h0, n, sem):
        return [pltpu.make_async_copy(src.at[:, pl.ds(128 * (h0 + j), 128)], dst.at[h0 + j], sem)
                for j in range(n)]

    def wait_heads(buf, h0, n, sem):
        dst = buf.at[pl.ds(h0, n)]
        pltpu.make_async_copy(dst, dst, sem).wait()

    def wq_copy(g, sem):
        a, b = wqg[g]
        cs = pl.ds(128 * a, 128 * (b - a))
        return pltpu.make_async_copy(wq_hbm.at[:, cs], wq_s.at[:, cs], sem)

    def kv_parts(i):
        return ((NM * i, NM), (NMAIN + i, 1))

    def kv_copies(i):
        out = []
        for h0, n in kv_parts(i):
            out.append(pltpu.make_async_copy(k_hbm.at[:, pl.ds(h0, n)], k_s.at[:, pl.ds(h0, n)], sem_kv.at[i]))
            out.append(pltpu.make_async_copy(v_hbm.at[:, pl.ds(h0, n)], v_s.at[:, pl.ds(h0, n)], sem_kv.at[i]))
        return out

    def wqt_copy(i):
        c0 = 128 * (NMAIN + i)
        if not isinstance(i, int):
            c0 = pl.multiple_of(c0, 128)
        return pltpu.make_async_copy(wq_hbm.at[:, pl.ds(c0, 128)], wqt_s.at[i], sem_kv.at[i])

    def start_kv(i):
        cps = [wqt_copy(i)] + kv_copies(i)
        for h0, n in kv_parts(i):
            cps += w_copies(wo_hbm, wo_s, h0, n, sem_kv.at[i])
        for cp in cps:
            cp.start()

    def wait_kv(i):
        wqt_copy(i).wait()
        for h0, n in kv_parts(i):
            wait_heads(wo_s, h0, n, sem_kv.at[i])
        for cp in kv_copies(i):
            cp.wait()

    def o_copy(p):
        return pltpu.make_async_copy(out_s.at[p], o_hbm.at[pl.ds(128 * p, 128)], sem_o)

    def fence():
        pl.semaphore_signal(bar_sem, 1)
        pl.semaphore_wait(bar_sem, 1)

    for k, step in enumerate(PLAN):
        for kind, idx in step["wait"]:
            if kind == "x":
                x_copy(idx, sem_p1.at[k]).start()
            else:
                wq_copy(idx, sem_p1.at[k]).start()
            fence()
    start_kv(0)
    fence()
    start_kv(1)

    acc_s[...] = jnp.zeros_like(acc_s)

    left = jax.lax.broadcasted_iota(jnp.int32, (64, 128), 1) < 64
    left1 = jax.lax.broadcasted_iota(jnp.int32, (1, 128), 1) < 64

    def to_u32(v):
        return pltpu.bitcast(v, U32)

    def to_bf(v):
        return pltpu.bitcast(v, BF)

    def make_xr(p):
        xr = x_s[128 * p:128 * (p + 1), DM:D].astype(F32)
        z = jnp.zeros((64, 64), F32)
        top = jnp.concatenate([z, xr[:64]], axis=1)
        bot = jnp.concatenate([xr[64:], z], axis=1)
        xr_s[p] = to_u32(jnp.concatenate([top, bot], axis=0).T.astype(BF))

    def wq_rows(h, r0, r1, tail):
        return wqt_s[h, r0:r1, :] if tail else wq_s[r0:r1, 128 * h:128 * (h + 1)]

    def make_wr(h, tail=False):
        wr = wq_rows(h, DM, D, tail)
        val = to_u32(jnp.concatenate([wr, wr], axis=0).T)
        if tail:
            wrt_s[...] = val
        else:
            wr_s[h] = val

    def mm_a(h, r0, nr, tail=False):
        return jnp.dot(x_s[r0:r0 + nr, 0:DM], wq_rows(h, 0, DM, tail), preferred_element_type=F32).astype(BF)

    def epi_a(h, r0, q, tail=False):
        wr2 = wrt_s[...] if tail else wr_s[h]
        for i in range(q.shape[0] // 128):
            p = r0 // 128 + i
            qt = to_u32(q[128 * i:128 * (i + 1), :].T)
            t1 = jnp.where(left, qt, wr2)
            t2 = jnp.where(left, wr2, qt)
            if tail:
                tt_s[p, 0] = t1
                tt_s[p, 1] = t2
            else:
                t_s[h, p, 0] = t1
                t_s[h, p, 1] = t2

    def st_a(h, r0, nr, tail=False):
        epi_a(h, r0, mm_a(h, r0, nr, tail), tail)

    def st_b(h, p, tail, late=False):
        if late:
            e = p - (NP - LATE // 128)
            t1, t2 = tt2_s[e, 0], tt2_s[e, 1]
        else:
            t1, t2 = (tt_s[p, 0], tt_s[p, 1]) if tail else (t_s[h, p, 0], t_s[h, p, 1])
        r1 = jnp.dot(k_s[2 * p, h], to_bf(t1), preferred_element_type=F32)
        r2 = jnp.dot(k_s[2 * p + 1, h], to_bf(t2), preferred_element_type=F32)
        return jnp.where(left, r1, r2), jnp.where(left, r2, r1).astype(BF)

    def st_r(p, sg):
        s_main, g = sg
        s = s_main + jnp.dot(g, to_bf(xr_s[p]), preferred_element_type=F32)
        m = jnp.max(s, axis=0, keepdims=True)
        e = jnp.exp2((s - m) * c)
        r = 1.0 / jnp.sum(e, axis=0, keepdims=True)
        rt = jnp.where(left1, r, 0.0)
        rb = jnp.where(left1, 0.0, r)
        return jnp.concatenate([(e * rt).astype(BF), (e * rb).astype(BF)], axis=0)

    def st_c(h, p, w):
        vp = v_s[2 * p:2 * p + 2, h].reshape(128, 128)
        return jax.lax.dot_general(vp, w, TN, preferred_element_type=F32).astype(BF)

    def st_d_mm(h, ot):
        rows = D // DSPLIT
        return [jnp.dot(wo_s[h, rows * r:rows * (r + 1), :], ot, preferred_element_type=F32)
                for r in range(DSPLIT)]

    def st_d_acc(p, prods, last, last_iter):
        rows = D // DSPLIT
        parts = []
        for r in range(DSPLIT):
            sl = slice(rows * r, rows * (r + 1))
            part = acc_s[p, sl] + prods[r]
            acc_s[p, sl] = part
            parts.append(part)
        if not last:
            return
        if p == NP - 1:
            @pl.when(last_iter)
            def _():
                out_s[p] = acc_s[p].astype(BF).T
                o_copy(p).start()
        else:
            out_s[p] = jnp.concatenate(parts, axis=0).astype(BF).T

            @pl.when(last_iter)
            def _():
                o_copy(p).start()

    pending = []
    for k, step in enumerate(PLAN):
        for kind, idx in step["wait"]:
            if kind == "x":
                x_copy(idx, sem_p1.at[k]).wait()
            else:
                wq_copy(idx, sem_p1.at[k]).wait()
        while pending:
            epi_a(*pending.pop(0))
        if step.get("xr"):
            for p in range(NP):
                make_xr(p)
        items = [(g, h, XCH[c0], XCH[c1] - XCH[c0])
                 for (g, c0, c1) in step["do"] for h in range(*wqg[g])]
        for n, (g, h, r0, nr) in enumerate(items):
            if ("w", g) in step["wait"]:
                make_wr(h)
            if h % NM == NM - 1:
                assert r0 == 0 and nr == M and k == len(PLAN) - 1
                nr = M - LATE
            if n == len(items) - 1 and k < len(PLAN) - 1:
                if nr > DEFER:
                    st_a(h, r0, nr - DEFER)
                r1 = r0 + nr - DEFER
                pending.append((h, r1, mm_a(h, r1, DEFER)))
            else:
                st_a(h, r0, nr)

    for i in range(2):
        q2_s[i] = to_u32(mm_a(NM * i + NM - 1, M - LATE, LATE))

    def p2_body(i, carry):
        wait_kv(i)
        last_iter = i == 1
        make_wr(i, tail=True)
        units = [(j, p) for j in range(16 - GL) for p in range(NP)]
        units += [(j, p) for p in range(NP) for j in range(16 - GL, 16)]
        n = len(units)
        vals = {}
        deferred = []
        for t in range(n + SKEW["D"]):
            if t == FENCE:
                fence()
                while deferred:
                    st_d_acc(*deferred.pop(0))
            if t < NP:
                st_a(i, 128 * t, 128, tail=True)
            if t == NP:
                q2 = to_bf(q2_s[i])
                wr2 = wr_s[NM * i + NM - 1]
                for e in range(LATE // 128):
                    qt = to_u32(q2[128 * e:128 * (e + 1), :].T)
                    tt2_s[e, 0] = jnp.where(left, qt, wr2)
                    tt2_s[e, 1] = jnp.where(left, wr2, qt)
            for s in ORDER:
                u = t - SKEW[s]
                if not 0 <= u < n:
                    continue
                j, p = units[u]
                h = _p2_head(i, j)
                if s == "B":
                    vals["B", u] = st_b(h, p, j == 1, j == 15 and p >= NP - LATE // 128)
                elif s == "R":
                    vals["R", u] = st_r(p, vals.pop(("B", u)))
                elif s == "C":
                    vals["C", u] = st_c(h, p, vals.pop(("R", u)))
                else:
                    args = (p, st_d_mm(h, vals.pop(("C", u))), j == 15, last_iter)
                    if t == FENCE - 1:
                        deferred.append(args)
                    else:
                        st_d_acc(*args)
        return carry

    jax.lax.fori_loop(0, 2, p2_body, 0)
    for p in range(NP):
        o_copy(p).wait()


@jax.jit
def pallas_standalone__mha_block_cached__near_ridge_kernel(x, k_cache, v_cache, wq, wo):
    out = pl.pallas_call(
        _kernel,
        in_specs=[pl.BlockSpec(memory_space=pl.ANY)] * 5,
        out_specs=pl.BlockSpec(memory_space=pl.ANY),
        out_shape=jax.ShapeDtypeStruct((M, D), BF),
        scratch_shapes=[
            pltpu.VMEM((M, D), BF),
            pltpu.VMEM((B, H, SK, DH), BF),
            pltpu.VMEM((B, H, SK, DH), BF),
            pltpu.VMEM((D, NMAIN * DH), BF),
            pltpu.VMEM((2, D, DH), BF),
            pltpu.VMEM((H, D, DH), BF),
            pltpu.VMEM((H, NP, 2, 64, 128), U32),
            pltpu.VMEM((NP, 2, 64, 128), U32),
            pltpu.VMEM((2, LATE // 2, 128), U32),
            pltpu.VMEM((LATE // 128, 2, 64, 128), U32),
            pltpu.VMEM((H, 64, 128), U32),
            pltpu.VMEM((64, 128), U32),
            pltpu.VMEM((NP, 64, 128), U32),
            pltpu.VMEM((NP, D, 128), F32),
            pltpu.VMEM((NP, 128, D), BF),
            pltpu.SemaphoreType.DMA((len(PLAN),)),
            pltpu.SemaphoreType.DMA((2,)),
            pltpu.SemaphoreType.DMA,
            pltpu.SemaphoreType.REGULAR,
        ],
        compiler_params=pltpu.CompilerParams(vmem_limit_bytes=100 * 1024 * 1024),
    )(x.reshape(M, D), k_cache, v_cache, wq, wo.T)
    return out.reshape(B, SQ, D)
```
